```python
import os as _os
_os.environ.setdefault("JAX_PLATFORMS", "cpu")
import jax
import jax.numpy as jnp

def _softmax(x, axis=-1):
    return jax.nn.softmax(x, axis=axis)
def _gelu(x):
    return jax.nn.gelu(x, approximate=True)
def _silu(x):
    return jax.nn.silu(x)
def _sigmoid(x):
    return jax.nn.sigmoid(x)
def _layernorm(x, axis=-1, eps=1e-5):
    m = jnp.mean(x, axis=axis, keepdims=True)
    v = jnp.var(x, axis=axis, keepdims=True)
    return (x - m) / jnp.sqrt(v + eps)
def _scatter_add(tgt, idx, src, axis=0):
    return tgt.at[idx].add(src)
def _segment_sum(src, seg, n):
    return jax.ops.segment_sum(src, seg, n)
class _Rng:
    def __init__(self, key):
        self._k = key
    def _next(self):
        self._k, sub = jax.random.split(self._k)
        return sub
    def normal(self, shape):
        return jax.random.normal(self._next(), shape, dtype=jnp.bfloat16)
    def randint(self, lo, hi, shape):
        return jax.random.randint(self._next(), shape, lo, hi, dtype=jnp.int32)
    def uniform(self, shape, lo=0.0, hi=1.0):
        return jax.random.uniform(self._next(), shape, jnp.bfloat16, lo, hi)
    def permutation(self, n):
        return jax.random.permutation(self._next(), n)


kernel_name = 'standalone__mha_block_cached__near_ridge'

def setup_inputs():
    _rng = _Rng(jax.random.key(int.from_bytes(__import__("os").urandom(4), "little")))
    _w = (lambda a: (lambda t: t.astype(jnp.bfloat16) if jnp.issubdtype(t.dtype, jnp.floating) else t)(jnp.asarray(a)))
    B, Sq, D = 8, 96, 576
    H, Sk, Dh = 32, 96, 128
    return {
        "x": _w((lambda *s: _rng.normal(s) * 0.8)(B, Sq, D)),
        "k_cache": _w((lambda *s: _rng.normal(s) * 0.8)(B, H, Sk, Dh)),
        "v_cache": _w((lambda *s: _rng.normal(s) * 0.05)(B, H, Sk, Dh)),
        "wq": _w((lambda *s: _rng.normal(s) * 0.8)(D, H * Dh) * (D ** -0.5)),
        "wo": _w((lambda *s: _rng.normal(s) * 0.05)(H * Dh, D) * ((H * Dh) ** -0.5)),
    }

def reference(x, k_cache, v_cache, wq, wo):
    B, Sq, D = x.shape
    H, Dh = 32, 128
    q = (lambda x, *d: x.transpose(*d))((x @ wq).reshape(B, Sq, H, Dh), 0, 2, 1, 3)
    scores = jnp.einsum("bhqd,bhkd->bhqk", q, k_cache) * (Dh ** -0.5)
    p = _softmax(scores, axis=-1)
    o = jnp.einsum("bhqk,bhkd->bhqd", p, v_cache)
    return (lambda x, *d: x.transpose(*d))(o, 0, 2, 1, 3).reshape(B, Sq, H * Dh) @ wo
```

```python
import jax
import jax.numpy as jnp
import jax.experimental.pallas as pl
import jax.experimental.pallas.tpu as pltpu

B, SQ, D, H, SK, DH = 8, 96, 576, 32, 96, 128
M = B * SQ
G = 4
NG = H // G
GW = G * DH
NT = M // 128
DM = 512
KT = ((DM, D - DM), (0, 128), (128, 128), (256, 128), (384, 128))
NK = len(KT)
LEAD = 2
LOOP = (1, 3)
EXP2_SCALE = (DH ** -0.5) * 1.4426950408889634
NT_DIMS = (((1,), (1,)), ((), ()))
f32, bf16 = jnp.float32, jnp.bfloat16


def _spread(ops, n):
    cuts = [(len(ops) * i + n - 1) // n for i in range(n + 1)]
    return [ops[cuts[i]:cuts[i + 1]] for i in range(n)]


def _needs(op):
    t, g = op[0], op[1]
    if t == "z":
        return [("x", g), ("wq0", g)]
    return [({"q": "wq", "o": "wo", "s": "k", "p": "v"}[t], g)]


def _build_schedule():
    prog = [("z", k) for k in range(NK)]
    prog += [("q", g, k, 0, 1) for g in range(1, LEAD) for k in range(NK)]
    bounds = []
    early_out = {3: 0, 4: 1, 5: 2, 7: 3}
    for g in range(NG):
        bounds.append(len(prog))
        has_q, has_o = g + LEAD < NG, g >= 1
        if has_q and has_o:
            qs = [("q", g + LEAD, k, 0, 1) for k in range(NK)]
            os_ = [("o", g - 1, n, 0, 1) for n in range(NT)]
            fill = [[(qs if ch == "q" else os_).pop(0) for ch in slot]
                    for slot in "oq,o,q,o,qo,q,o,qo".split(",")]
        elif has_q:
            fill = _spread([("q", g + LEAD, k, j, 2) for k in range(NK) for j in range(2)], B)
        elif g < NG - 1:
            fill = _spread([("o", g - 1, n, j, 2) for n in range(NT) for j in range(2)], B)
        else:
            fill = _spread([("o", g - 1, n, 0, 1) for n in range(NT)], B)
            for b, n in early_out.items():
                fill[b] = fill[b] + [("o", g, n, 0, 1)]
        for b in range(B):
            prog += [("s", g, b)] + fill[b] + [("p", g, b)]
    flush = len(prog)
    prog += [("o", NG - 1, n, 0, 1) for n in range(len(early_out), NT)]
    waits = [0, 1, 2, 3, NK] + [bounds[g] for g in (0, 1, 2, 3, 5)]
    sets, seen = [], []
    for lo, hi in zip(waits, waits[1:] + [len(prog)]):
        cur = []
        for op in prog[lo:hi]:
            for d in _needs(op):
                if d not in seen:
                    seen.append(d)
                    cur.append(d)
        sets.append(cur)
    return prog, bounds, waits, sets, flush


def _kernel(x_hbm, k_hbm, v_hbm, wq_hbm, wo_hbm, o_hbm,
            x_s, k_s, v_s, wq_s, wo_s, qacc, q_s, o_s, acc, out_s, fence_s, sem):
    prog, bounds, waits, sets, flush = _build_schedule()

    def copy_in(d, j, dg=0):
        t, g = d[0], d[1] + dg
        if t == "x":
            k0, kn = KT[g]
            src, dst = x_hbm.at[:, k0:k0 + kn], x_s.at[:, k0:k0 + kn]
        elif t == "wq0":
            k0, kn = KT[g]
            src, dst = wq_hbm.at[k0:k0 + kn, 0:GW], wq_s.at[0, k0:k0 + kn]
        elif t in ("wq", "wo"):
            a, s = (wq_hbm, wq_s) if t == "wq" else (wo_hbm, wo_s)
            src, dst = a.at[:, pl.ds(pl.multiple_of(g * GW, GW), GW)], s.at[g]
        else:
            a, s = (k_hbm, k_s) if t == "k" else (v_hbm, v_s)
            src, dst = a.at[:, pl.ds(g * G, G)], s.at[g]
        return pltpu.make_async_copy(src, dst, sem.at[j + dg])

    def copy_out(n):
        rows = slice(n * 128, (n + 1) * 128)
        return pltpu.make_async_copy(out_s.at[rows], o_hbm.at[rows], sem.at[len(sets)])

    fence = pltpu.make_async_copy(k_hbm.at[0, 0, 0:16], fence_s, sem.at[len(sets) + 1])

    def z_piece(dg, j):
        k0, kn = KT[j]
        r = jnp.dot(x_s[:, k0:k0 + kn], wq_s[0, k0:k0 + kn, :], preferred_element_type=f32)
        if j == 0:
            qacc[...] = r
        elif j < NK - 1:
            qacc[...] += r
        else:
            q_s[0] = (qacc[...] + r).astype(bf16)

    def q_piece(dg, g0, k, j, n):
        g = g0 + dg
        rs = slice(j * M // n, (j + 1) * M // n)
        if k == 0:
            qacc[rs] = jnp.dot(x_s[rs, DM:D], wq_s[g, DM:D, :], preferred_element_type=f32)
        else:
            hs = slice((k - 1) * DH, k * DH)
            r = jnp.dot(x_s[rs, 0:DM], wq_s[g, 0:DM, hs], preferred_element_type=f32)
            q_s[g, rs, hs] = (qacc[rs, hs] + r).astype(bf16)

    def o_piece(dg, g0, n, j, nn):
        g = g0 + dg
        rs = slice(j * D // nn, (j + 1) * D // nn)
        cs = slice(n * 128, (n + 1) * 128)
        r = jax.lax.dot_general(wo_s[g, rs], o_s[g, cs, :], NT_DIMS, preferred_element_type=f32)
        if g0 < NG - 1:
            acc[rs, cs] += r
        else:
            for r0 in range(0, D, 128):
                r1 = min(D, r0 + 128)
                out_s[cs, r0:r1] = (acc[r0:r1, cs] + r[r0:r1]).T.astype(bf16)
            copy_out(n).start()

    live = {}

    def s_piece(dg, g0, b):
        g = g0 + dg
        res = []
        for h in range(G):
            q = q_s[g, b * SQ:(b + 1) * SQ, h * DH:(h + 1) * DH]
            s = jax.lax.dot_general(q, k_s[g, b, h], NT_DIMS, preferred_element_type=f32)
            m = jnp.max(s, axis=-1, keepdims=True)
            p = jnp.exp2((s - m) * EXP2_SCALE)
            l = jnp.sum(p, axis=-1, keepdims=True)
            r = pl.reciprocal(l, approx=True)
            r = r * (2.0 - l * r)
            res.append((p.astype(bf16), r))
        live[g0, b] = res

    def p_piece(dg, g0, b):
        g = g0 + dg
        for h, (p, r) in enumerate(live.pop((g0, b))):
            o = jnp.dot(p, v_s[g, b, h], preferred_element_type=f32) * r
            o_s[g, b * SQ:(b + 1) * SQ, h * DH:(h + 1) * DH] = o.astype(bf16)

    piece = dict(z=z_piece, q=q_piece, o=o_piece, s=s_piece, p=p_piece)

    def run(lo, hi, dg=0):
        for i in range(lo, hi):
            if i in waits:
                j = waits.index(i)
                for d in sets[j]:
                    copy_in(d, j, dg).wait()
            if i == flush:
                fence.wait()
            piece[prog[i][0]](dg, *prog[i][1:])

    for j, cur in enumerate(sets):
        for d in cur:
            copy_in(d, j).start()
    fence.start()
    acc[...] = jnp.zeros(acc.shape, f32)

    l0, l1 = LOOP
    run(0, bounds[l0])
    jax.lax.fori_loop(0, l1 - l0, lambda i, _: run(bounds[l0], bounds[l0 + 1], i), None)
    run(bounds[l1], len(prog))
    for n in range(NT):
        copy_out(n).wait()


@jax.jit
def pallas_standalone__mha_block_cached__near_ridge_kernel(
    x: jax.Array,
    k_cache: jax.Array,
    v_cache: jax.Array,
    wq: jax.Array,
    wo: jax.Array,
):
    assert x.shape == (B, SQ, D) and k_cache.shape == v_cache.shape == (B, H, SK, DH)
    hbm = pl.BlockSpec(memory_space=pltpu.HBM)
    num_sems = len(_build_schedule()[3]) + 2
    out = pl.pallas_call(
        _kernel,
        in_specs=[hbm] * 5,
        out_specs=hbm,
        out_shape=jax.ShapeDtypeStruct((M, D), x.dtype),
        scratch_shapes=[
            pltpu.VMEM((M, D), bf16),
            pltpu.VMEM((NG, B, G, SK, DH), bf16),
            pltpu.VMEM((NG, B, G, SK, DH), bf16),
            pltpu.VMEM((NG, D, GW), bf16),
            pltpu.VMEM((NG, D, GW), bf16),
            pltpu.VMEM((M, GW), f32),
            pltpu.VMEM((NG, M, GW), bf16),
            pltpu.VMEM((NG, M, GW), bf16),
            pltpu.VMEM((D, M), f32),
            pltpu.VMEM((M, D), bf16),
            pltpu.VMEM((16, DH), bf16),
            pltpu.SemaphoreType.DMA((num_sems,)),
        ],
        compiler_params=pltpu.CompilerParams(vmem_limit_bytes=100 * 1024 * 1024),
    )(x.reshape(M, D), k_cache, v_cache, wq, wo.T)
    return out.reshape(B, SQ, D)
```

```python
import jax
import jax.numpy as jnp
import jax.experimental.pallas as pl
import jax.experimental.pallas.tpu as pltpu

B, SQ, D, H, SK, DH = 8, 96, 576, 32, 96, 128
M = B * SQ
G = 4
NG = H // G
GW = G * DH
NT = M // 128
DM = 512
KT = ((DM, D - DM), (0, 128), (128, 128), (256, 128), (384, 128))
NK = len(KT)
LEAD = 2
LOOP = (1, 3)
EXP2_SCALE = (DH ** -0.5) * 1.4426950408889634
NT_DIMS = (((1,), (1,)), ((), ()))
f32, bf16 = jnp.float32, jnp.bfloat16


def _spread(ops, n):
    cuts = [(len(ops) * i + n - 1) // n for i in range(n + 1)]
    return [ops[cuts[i]:cuts[i + 1]] for i in range(n)]


def _needs(op):
    t, g = op[0], op[1]
    if t == "z":
        return [("x", g), ("wq0", g)]
    return [({"q": "wq", "o": "wo", "s": "k", "p": "v"}[t], g)]


def _build_schedule():
    prog = [("z", k) for k in range(NK)]
    prog += [("q", g, k, 0, 1) for g in range(1, LEAD) for k in range(NK)]
    bounds = []
    for g in range(NG):
        bounds.append(len(prog))
        has_q, has_o = g + LEAD < NG, g >= 1
        if has_q and has_o:
            qs = [("q", g + LEAD, k, 0, 1) for k in range(NK)]
            os_ = [("o", g - 1, n, 0, 1) for n in range(NT)]
            fill = [[(qs if ch == "q" else os_).pop(0) for ch in slot]
                    for slot in "oq,o,q,o,qo,q,o,qo".split(",")]
        elif has_q:
            fill = _spread([("q", g + LEAD, k, j, 2) for k in range(NK) for j in range(2)], B)
        elif g < NG - 1:
            fill = _spread([("o", g - 1, n, j, 2) for n in range(NT) for j in range(2)], B)
        else:
            fill = [[("o", g - dg, n, 0, 1)] for dg, n in
                    ((1, 0), (1, 1), (1, 2), (0, 0), (0, 1), (1, 3), (1, 4), (0, 3))]
            fill[5].append(("o", g, 2, 0, 1))
        for b in range(B):
            prog += [("s", g, b)] + fill[b] + [("p", g, b)]
    prog.append(("o", NG - 2, NT - 1, 0, 1))
    flush = len(prog)
    prog += [("o", NG - 1, n, 0, 1) for n in range(4, NT)]
    waits = [0, 1, 2, 3, NK] + [bounds[g] for g in (0, 1, 2, 3, 5)]
    sets, seen = [], []
    for lo, hi in zip(waits, waits[1:] + [len(prog)]):
        cur = []
        for op in prog[lo:hi]:
            for d in _needs(op):
                if d not in seen:
                    seen.append(d)
                    cur.append(d)
        sets.append(cur)
    return prog, bounds, waits, sets, flush


def _kernel(x_hbm, k_hbm, v_hbm, wq_hbm, wo_hbm, o_hbm,
            x_s, k_s, v_s, wq_s, wo_s, qacc, q_s, o_s, acc, out_s, fence_s, sem):
    prog, bounds, waits, sets, flush = _build_schedule()

    def copy_in(d, j, dg=0):
        t, g = d[0], d[1] + dg
        if t == "x":
            k0, kn = KT[g]
            src, dst = x_hbm.at[:, k0:k0 + kn], x_s.at[:, k0:k0 + kn]
        elif t == "wq0":
            k0, kn = KT[g]
            src, dst = wq_hbm.at[k0:k0 + kn, 0:GW], wq_s.at[0, k0:k0 + kn]
        elif t in ("wq", "wo"):
            a, s = (wq_hbm, wq_s) if t == "wq" else (wo_hbm, wo_s)
            src, dst = a.at[:, pl.ds(pl.multiple_of(g * GW, GW), GW)], s.at[g]
        else:
            a, s = (k_hbm, k_s) if t == "k" else (v_hbm, v_s)
            src, dst = a.at[:, pl.ds(g * G, G)], s.at[g]
        return pltpu.make_async_copy(src, dst, sem.at[j + dg])

    def copy_out(n):
        rows = slice(n * 128, (n + 1) * 128)
        return pltpu.make_async_copy(out_s.at[rows], o_hbm.at[rows], sem.at[len(sets)])

    fence = pltpu.make_async_copy(k_hbm.at[0, 0, 0:16], fence_s, sem.at[len(sets) + 1])

    def z_piece(dg, j):
        k0, kn = KT[j]
        r = jnp.dot(x_s[:, k0:k0 + kn], wq_s[0, k0:k0 + kn, :], preferred_element_type=f32)
        if j == 0:
            qacc[...] = r
        elif j < NK - 1:
            qacc[...] += r
        else:
            q_s[0] = (qacc[...] + r).astype(bf16)

    def q_piece(dg, g0, k, j, n):
        g = g0 + dg
        rs = slice(j * M // n, (j + 1) * M // n)
        if k == 0:
            qacc[rs] = jnp.dot(x_s[rs, DM:D], wq_s[g, DM:D, :], preferred_element_type=f32)
        else:
            hs = slice((k - 1) * DH, k * DH)
            r = jnp.dot(x_s[rs, 0:DM], wq_s[g, 0:DM, hs], preferred_element_type=f32)
            q_s[g, rs, hs] = (qacc[rs, hs] + r).astype(bf16)

    def o_piece(dg, g0, n, j, nn):
        g = g0 + dg
        rs = slice(j * D // nn, (j + 1) * D // nn)
        cs = slice(n * 128, (n + 1) * 128)
        r = jax.lax.dot_general(wo_s[g, rs], o_s[g, cs, :], NT_DIMS, preferred_element_type=f32)
        if g0 < NG - 1:
            acc[rs, cs] += r
        else:
            for r0 in range(0, D, 128):
                r1 = min(D, r0 + 128)
                out_s[cs, r0:r1] = (acc[r0:r1, cs] + r[r0:r1]).T.astype(bf16)
            copy_out(n).start()

    live = {}

    def s_piece(dg, g0, b):
        g = g0 + dg
        res = []
        for h in range(G):
            q = q_s[g, b * SQ:(b + 1) * SQ, h * DH:(h + 1) * DH]
            s = jax.lax.dot_general(q, k_s[g, b, h], NT_DIMS, preferred_element_type=f32)
            m = jnp.max(s, axis=-1, keepdims=True)
            p = jnp.exp2((s - m) * EXP2_SCALE)
            l = jnp.sum(p, axis=-1, keepdims=True)
            r = pl.reciprocal(l, approx=True)
            r = r * (2.0 - l * r)
            res.append((p.astype(bf16), r))
        live[g0, b] = res

    def p_piece(dg, g0, b):
        g = g0 + dg
        for h, (p, r) in enumerate(live.pop((g0, b))):
            o = jnp.dot(p, v_s[g, b, h], preferred_element_type=f32) * r
            o_s[g, b * SQ:(b + 1) * SQ, h * DH:(h + 1) * DH] = o.astype(bf16)

    piece = dict(z=z_piece, q=q_piece, o=o_piece, s=s_piece, p=p_piece)

    def run(lo, hi, dg=0):
        for i in range(lo, hi):
            if i in waits:
                j = waits.index(i)
                for d in sets[j]:
                    copy_in(d, j, dg).wait()
            if i == flush:
                fence.wait()
            piece[prog[i][0]](dg, *prog[i][1:])

    for j, cur in enumerate(sets):
        for d in cur:
            copy_in(d, j).start()
    fence.start()
    acc[...] = jnp.zeros(acc.shape, f32)

    l0, l1 = LOOP
    run(0, bounds[l0])
    jax.lax.fori_loop(0, l1 - l0, lambda i, _: run(bounds[l0], bounds[l0 + 1], i), None)
    run(bounds[l1], len(prog))
    for n in range(NT):
        copy_out(n).wait()


@jax.jit
def pallas_standalone__mha_block_cached__near_ridge_kernel(
    x: jax.Array,
    k_cache: jax.Array,
    v_cache: jax.Array,
    wq: jax.Array,
    wo: jax.Array,
):
    assert x.shape == (B, SQ, D) and k_cache.shape == v_cache.shape == (B, H, SK, DH)
    hbm = pl.BlockSpec(memory_space=pltpu.HBM)
    num_sems = len(_build_schedule()[3]) + 2
    out = pl.pallas_call(
        _kernel,
        in_specs=[hbm] * 5,
        out_specs=hbm,
        out_shape=jax.ShapeDtypeStruct((M, D), x.dtype),
        scratch_shapes=[
            pltpu.VMEM((M, D), bf16),
            pltpu.VMEM((NG, B, G, SK, DH), bf16),
            pltpu.VMEM((NG, B, G, SK, DH), bf16),
            pltpu.VMEM((NG, D, GW), bf16),
            pltpu.VMEM((NG, D, GW), bf16),
            pltpu.VMEM((M, GW), f32),
            pltpu.VMEM((NG, M, GW), bf16),
            pltpu.VMEM((NG, M, GW), bf16),
            pltpu.VMEM((D, M), f32),
            pltpu.VMEM((M, D), bf16),
            pltpu.VMEM((16, DH), bf16),
            pltpu.SemaphoreType.DMA((num_sems,)),
        ],
        compiler_params=pltpu.CompilerParams(vmem_limit_bytes=100 * 1024 * 1024),
    )(x.reshape(M, D), k_cache, v_cache, wq, wo.T)
    return out.reshape(B, SQ, D)
```
